```python
import jax
import jax.numpy as jnp

def _softmax(x, axis=-1):
    return jax.nn.softmax(x, axis=axis)
def _gelu(x):
    return jax.nn.gelu(x, approximate=True)
def _silu(x):
    return jax.nn.silu(x)
def _sigmoid(x):
    return jax.nn.sigmoid(x)
def _layernorm(x, axis=-1, eps=1e-5):
    m = jnp.mean(x, axis=axis, keepdims=True)
    v = jnp.var(x, axis=axis, keepdims=True)
    return (x - m) / jnp.sqrt(v + eps)
def _scatter_add(tgt, idx, src, axis=0):
    return tgt.at[idx].add(src)
def _segment_sum(src, seg, n):
    return jax.ops.segment_sum(src, seg, n)
class _Rng:
    def __init__(self, key):
        self._k = key
    def _next(self):
        self._k, sub = jax.random.split(self._k)
        return sub
    def normal(self, shape):
        return jax.random.normal(self._next(), shape, dtype=jnp.bfloat16)
    def randint(self, lo, hi, shape):
        return jax.random.randint(self._next(), shape, lo, hi, dtype=jnp.int32)
    def uniform(self, shape, lo=0.0, hi=1.0):
        return jax.random.uniform(self._next(), shape, jnp.bfloat16, lo, hi)
    def permutation(self, n):
        return jax.random.permutation(self._next(), n)


kernel_name = 'interleave_layers__sliding_local_dilated__glu_gated_bilinear__prompt'

def setup_inputs():
    _rng = _Rng(jax.random.key(int.from_bytes(__import__("os").urandom(4), "little")))
    _w = (lambda a: (lambda t: t.astype(jnp.bfloat16) if jnp.issubdtype(t.dtype, jnp.floating) else t)(jnp.asarray(a)))
    def _A_setup():
        B, S, D = 1, 2048, 576
        return {
            "x": _w((lambda *s: _rng.normal(s) * 0.05)(B, S, D)),
            "wqkv": _w((lambda *s: _rng.normal(s) * 0.05)(D, 3 * D)),
            "wo": _w((lambda *s: _rng.normal(s) * 0.05)(D, D)),
        }
    _A_in = _A_setup()

    def _B_setup():
        B, S, D, F = 1, 2048, 576, 4608
        return {
            "x": _w((lambda *s: _rng.normal(s) * 0.05)(B, S, D)),
            "w_gate": _w((lambda *s: _rng.normal(s) * 0.05)(D, F) * (D ** -0.5)),
            "w_up": _w((lambda *s: _rng.normal(s) * 0.05)(D, F) * (D ** -0.5)),
            "w_down": _w((lambda *s: _rng.normal(s) * 0.05)(F, D) * (F ** -0.5)),
        }
    _B_in = _B_setup()

    return {
        "A_x": _A_in["x"],
        "A_wqkv": _A_in["wqkv"],
        "A_wo": _A_in["wo"],
        "B_x": _B_in["x"],
        "B_w_gate": _B_in["w_gate"],
        "B_w_up": _B_in["w_up"],
        "B_w_down": _B_in["w_down"],
    }

def reference(A_x, A_wqkv, A_wo, B_x, B_w_gate, B_w_up, B_w_down):
    def _A_ref(x, wqkv, wo):
        B, S, D = x.shape
        H = 32; Dh = D // H
        W, dil = 8, 2
        qkv = (lambda x, *d: x.transpose(*d))((x @ wqkv).reshape(B, S, 3, H, Dh), 2, 0, 3, 1, 4)
        q, k, v = qkv[0], qkv[1], qkv[2]
        scale = Dh ** -0.5
        pos = jnp.arange(S)
        off = jnp.arange(W) * dil
        idx = pos[:, None] - off[None, :]
        mask = idx >= 0
        idx_c = jnp.where(mask, idx, 0).reshape(-1)
        kg = k[:, :, idx_c, :].reshape(B, H, S, W, Dh)
        vg = v[:, :, idx_c, :].reshape(B, H, S, W, Dh)
        logits = jnp.einsum("bhsd,bhswd->bhsw", q, kg) * scale
        logits = jnp.where(mask[None, None, :, :], logits, -1e9)
        attn = _softmax(logits, axis=-1)
        o = jnp.einsum("bhsw,bhswd->bhsd", attn, vg)
        return (lambda x, *d: x.transpose(*d))(o, 0, 2, 1, 3).reshape(B, S, D) @ wo

    def _B_ref(x, w_gate, w_up, w_down):
        g = jnp.einsum("bsd,df->bsf", x, w_gate)
        u = jnp.einsum("bsd,df->bsf", x, w_up)
        h = g * u
        return jnp.einsum("bsf,fd->bsd", h, w_down)

    x = A_x
    x = x + _A_ref(_layernorm(x, axis=-1), A_wqkv, A_wo)
    x = x + _B_ref(_layernorm(x, axis=-1), B_w_gate, B_w_up, B_w_down)
    x = x + _A_ref(_layernorm(x, axis=-1), A_wqkv, A_wo)
    x = x + _B_ref(_layernorm(x, axis=-1), B_w_gate, B_w_up, B_w_down)
    return x
```

```python
import numpy as np
import jax
import jax.numpy as jnp
from jax import lax
import jax.experimental.pallas as pl
import jax.experimental.pallas.tpu as pltpu

S, D, F, H, DH, W, DIL = 2048, 576, 4608, 32, 18, 8, 2
DP = 640
HALO = 16
LOG2E = 1.4426950408889634
NT_DIMS = (((1,), (1,)), ((), ()))

def make(TM=512, FC=1152, skip=()):
    NT = S // TM
    NF = F // FC

    def kernel(x_ref, wqkv_hbm, wo_hbm, wg_hbm, wu_hbm, wd_hbm, o_ref,
               wqkv_raw, wo_raw, wqkv_p, wo_p, wg, wu, wd, kv, acc, xn_s, sems):
        i = pl.program_id(0)

        def cp_qkv():
            return pltpu.make_async_copy(wqkv_hbm, wqkv_raw, sems.at[0])
        def cp_wo():
            return pltpu.make_async_copy(wo_hbm, wo_raw, sems.at[1])
        def cp_g(c):
            return pltpu.make_async_copy(wg_hbm.at[:, pl.ds(c * FC, FC)], wg.at[c], sems.at[2 + 3 * c])
        def cp_u(c):
            return pltpu.make_async_copy(wu_hbm.at[:, pl.ds(c * FC, FC)], wu.at[c], sems.at[3 + 3 * c])
        def cp_d(c):
            return pltpu.make_async_copy(wd_hbm.at[:, pl.ds(c * FC, FC)], wd.at[c], sems.at[4 + 3 * c])

        @pl.when(i == 0)
        def _():
            cp_qkv().start()
            cp_wo().start()
            for c in range(NF):
                cp_g(c).start(); cp_u(c).start(); cp_d(c).start()
            r = lax.broadcasted_iota(jnp.int32, (D, DP), 0)
            cc = lax.broadcasted_iota(jnp.int32, (D, DP), 1)
            p = jnp.where((r == (cc % H) * DH + cc // H) & (cc < D), 1.0, 0.0).astype(jnp.bfloat16)
            kv[:, pl.ds(TM, HALO), :] = jnp.zeros((2, HALO, 2 * DP), jnp.float32)
            cp_qkv().wait()
            for t in range(3):
                wqkv_p[:, t * DP:(t + 1) * DP] = jnp.dot(
                    wqkv_raw[:, t * D:(t + 1) * D], p, preferred_element_type=jnp.float32).astype(jnp.bfloat16)
            cp_wo().wait()
            wo_p[...] = jnp.dot(wo_raw[...].astype(jnp.float32).T.astype(jnp.bfloat16), p,
                                preferred_element_type=jnp.float32).astype(jnp.bfloat16)

        def ln_t(xt):
            m = jnp.mean(xt, axis=0, keepdims=True)
            xc = xt - m
            v = jnp.mean(xc * xc, axis=0, keepdims=True)
            xn = xc * lax.rsqrt(v + 1e-5)
            if "tr" in skip:
                return jnp.broadcast_to(xn[0:1, 0:1], (TM, D)).astype(jnp.bfloat16)
            return xn.T.astype(jnp.bfloat16)

        def layer(l, carry):
            kvl = kv.at[l]
            kvl[pl.ds(0, HALO), :] = kvl[pl.ds(TM, HALO), :]
            xn = ln_t(acc[...])
            qkv = jnp.dot(xn, wqkv_p[...], preferred_element_type=jnp.float32)
            q = qkv[:, :DP] * (DH ** -0.5 * LOG2E)
            kvl[pl.ds(HALO, TM), :] = qkv[:, DP:]
            if "attn" in skip:
                o = q
            else:
                pos = i * TM + lax.broadcasted_iota(jnp.int32, (TM, 128), 0)
                ls = []
                for w in range(W):
                    kw = kvl[pl.ds(HALO - DIL * w, TM), 0:DP]
                    pr = q * kw
                    t = (pr[:, 0:128] + pr[:, 128:256]) + (pr[:, 256:384] + pr[:, 384:512]) + pr[:, 512:640]
                    t = t + pltpu.roll(t, 64, 1)
                    t = t + pltpu.roll(t, 32, 1)
                    if w > 0:
                        t = jnp.where(pos >= DIL * w, t, -1e9)
                    ls.append(t)
                m = ls[0]
                for w in range(1, W):
                    m = jnp.maximum(m, ls[w])
                es = [jnp.exp2(t - m) for t in ls]
                den = es[0]
                for w in range(1, W):
                    den = den + es[w]
                inv = 1.0 / den
                o = None
                for w in range(W):
                    vw = kvl[pl.ds(HALO - DIL * w, TM), DP:2 * DP]
                    pw = es[w] * inv
                    pw5 = jnp.concatenate([pw] * 5, axis=1)
                    o = pw5 * vw if o is None else o + pw5 * vw
            acc[...] += lax.dot_general(wo_p[...], o.astype(jnp.bfloat16), NT_DIMS, preferred_element_type=jnp.float32)
            xn_s[...] = ln_t(acc[...])

            def fbody(c, carry):
                @pl.when((i == 0) & (l == 0))
                def _():
                    cp_g(c).wait()
                    cp_u(c).wait(); cp_d(c).wait()
                xb = xn_s[...]
                g = jnp.dot(xb, wg[c], preferred_element_type=jnp.float32)
                u = jnp.dot(xb, wu[c], preferred_element_type=jnp.float32)
                h = (g * u).astype(jnp.bfloat16)
                acc[...] += lax.dot_general(wd[c], h, NT_DIMS, preferred_element_type=jnp.float32)
                return carry
            lax.fori_loop(0, NF, fbody, 0)
            return carry

        acc[...] = x_ref[...].astype(jnp.float32)
        lax.fori_loop(0, 2, layer, 0)
        o_ref[...] = acc[...].astype(o_ref.dtype)

    def fn(A_x, A_wqkv, A_wo, B_x, B_w_gate, B_w_up, B_w_down):
        xt = A_x.reshape(S, D).T
        hbm = pl.BlockSpec(memory_space=pltpu.MemorySpace.HBM)
        out = pl.pallas_call(
            kernel,
            grid=(NT,),
            in_specs=[pl.BlockSpec((D, TM), lambda i: (0, i))] + [hbm] * 5,
            out_specs=pl.BlockSpec((D, TM), lambda i: (0, i)),
            out_shape=jax.ShapeDtypeStruct((D, S), jnp.bfloat16),
            scratch_shapes=[
                pltpu.VMEM((D, 3 * D), jnp.bfloat16),
                pltpu.VMEM((D, D), jnp.bfloat16),
                pltpu.VMEM((D, 3 * DP), jnp.bfloat16),
                pltpu.VMEM((D, DP), jnp.bfloat16),
                pltpu.VMEM((NF, D, FC), jnp.bfloat16),
                pltpu.VMEM((NF, D, FC), jnp.bfloat16),
                pltpu.VMEM((NF, D, FC), jnp.bfloat16),
                pltpu.VMEM((2, HALO + TM, 2 * DP), jnp.float32),
                pltpu.VMEM((D, TM), jnp.float32),
                pltpu.VMEM((TM, D), jnp.bfloat16),
                pltpu.SemaphoreType.DMA((2 + 3 * NF,)),
            ],
            compiler_params=pltpu.CompilerParams(
                dimension_semantics=("arbitrary",),
                vmem_limit_bytes=100 * 1024 * 1024),
        )(xt, A_wqkv, A_wo, B_w_gate, B_w_up, B_w_down.T)
        return out.T.reshape(1, S, D)
    return fn


_impl = make(512, 1152)


@jax.jit
def pallas_interleave_layers__sliding_local_dilated__glu_gated_bilinear__prompt_kernel(
    A_x: jax.Array,
    A_wqkv: jax.Array,
    A_wo: jax.Array,
    B_x: jax.Array,
    B_w_gate: jax.Array,
    B_w_up: jax.Array,
    B_w_down: jax.Array,
):
    return _impl(A_x, A_wqkv, A_wo, B_x, B_w_gate, B_w_up, B_w_down)
```

```python
import numpy as np
import jax
import jax.numpy as jnp
from jax import lax
import jax.experimental.pallas as pl
import jax.experimental.pallas.tpu as pltpu

S, D, F, H, DH, W, DIL = 2048, 576, 4608, 32, 18, 8, 2
DP = 640
HALO = 16
LOG2E = 1.4426950408889634
GROUPS = ([(0, d) for d in range(16)] + [(1, d) for d in range(16)] + [(0, 16), (0, 17), (1, 16), (1, 17)]
          + [(2, d) for d in range(18)] + [None, None])
NT_DIMS = (((1,), (1,)), ((), ()))

def make(TM=512, FC=1152, order="FA", NS=1, flags=None):
    NT = S // TM
    NF = F // FC
    TA = -(-TM // (NF * 16)) * 16
    NJ = 2 * NT

    def tile_of(j):
        return (j // 4) * 2 + j % 2
    def layer_of(j):
        return (j // 2) % 2

    def kernel(x_hbm, wqkv_hbm, wo_hbm, wg_hbm, wu_hbm, wd_hbm, o_hbm,
               xin, xout, wqkv_raw, wo_raw, wqkv_p, wo_p, wg, wu, wd, q_s, kv, acc, xn1, xn2, o_s, wt, sems):
        def cp_qkv():
            return pltpu.make_async_copy(wqkv_hbm, wqkv_raw, sems.at[0])
        def cp_wo():
            return pltpu.make_async_copy(wo_hbm, wo_raw, sems.at[1])
        def cp_g(c):
            return pltpu.make_async_copy(wg_hbm.at[:, pl.ds(c * FC, FC)], wg.at[c], sems.at[2 + 3 * c])
        def cp_u(c):
            return pltpu.make_async_copy(wu_hbm.at[:, pl.ds(c * FC, FC)], wu.at[c], sems.at[3 + 3 * c])
        def cp_d(c):
            return pltpu.make_async_copy(wd_hbm.at[:, pl.ds(c * FC, FC)], wd.at[c], sems.at[4 + 3 * c])
        def cp_x(t):
            return pltpu.make_async_copy(x_hbm.at[:, pl.ds(pl.multiple_of(t * TM, TM), TM)], xin.at[t], sems.at[2 + 3 * NF + t])
        def cp_o(t):
            return pltpu.make_async_copy(xout.at[t], o_hbm.at[:, pl.ds(pl.multiple_of(t * TM, TM), TM)], sems.at[2 + 3 * NF + NT + t])

        cp_x(0).start()
        cp_qkv().start()
        cp_wo().start()
        for t in range(1, NT):
            cp_x(t).start()
        for c in range(NF):
            cp_g(c).start(); cp_u(c).start(); cp_d(c).start()
        kv[:, :, pl.ds(TM, HALO), :] = jnp.zeros((2, 10, HALO, 128), jnp.float32)

        def ln_t(xt):
            m = jnp.mean(xt, axis=0, keepdims=True)
            xc = xt - m
            v = jnp.mean(xc * xc, axis=0, keepdims=True)
            xn = xc * lax.rsqrt(v + 1e-5)
            return xn.T.astype(jnp.bfloat16)

        def ln1(j):
            xn1[...] = ln_t(acc[tile_of(j)])
        def ln2(j):
            xn2[...] = ln_t(acc[tile_of(j)])
        def qkv_mm(j):
            kvl = kv.at[layer_of(j)]
            kvl[:, pl.ds(0, HALO), :] = kvl[:, pl.ds(TM, HALO), :]
            qkv = lax.dot_general(xn1[...], wqkv_p[...], NT_DIMS, preferred_element_type=jnp.float32)
            sc = DH ** -0.5 * LOG2E
            q_s[:, 0:512] = qkv[:, 0:512] * sc
            lane = lax.broadcasted_iota(jnp.int32, (TM, 128), 1)
            q_s[:, 512:640] = jnp.where(lane >= 64, pltpu.roll(qkv[:, 1024:1152], 64, 1) * sc, 0.0)
            for b in range(10):
                kvl[b, pl.ds(HALO, TM), :] = qkv[:, 512 + b * 128:512 + (b + 1) * 128]
        def wo_mm(j):
            acc[tile_of(j)] += lax.dot_general(wo_p[...], o_s[...], NT_DIMS, preferred_element_type=jnp.float32)

        def attn(j, r0, n):
            kvl = kv.at[layer_of(j), :, pl.ds(pl.multiple_of(r0, 8), n + HALO)]
            q = q_s[pl.ds(r0, n), :]
            pos = tile_of(j) * TM + r0 + lax.broadcasted_iota(jnp.int32, (n, 128), 0)
            ls = []
            for w in range(W):
                pr = [q[:, b * 128:(b + 1) * 128] * kvl[b, pl.ds(HALO - DIL * w, n), :] for b in range(5)]
                t = (pr[0] + pr[1]) + (pr[2] + pr[3]) + pr[4]
                t = t + pltpu.roll(t, 64, 1)
                t = t + pltpu.roll(t, 32, 1)
                if w > 0:
                    t = jnp.where(pos >= DIL * w, t, -1e9)
                ls.append(t)
            m = ls[0]
            for w in range(1, W):
                m = jnp.maximum(m, ls[w])
            es = [jnp.exp2(t - m) for t in ls]
            den = es[0]
            for w in range(1, W):
                den = den + es[w]
            inv = 1.0 / den
            for b in range(5):
                o = None
                for w in range(W):
                    t = es[w] * kvl[5 + b, pl.ds(HALO - DIL * w, n), :]
                    o = t if o is None else o + t
                o_s[pl.ds(r0, n), b * 128:(b + 1) * 128] = (o * inv).astype(jnp.bfloat16)

        def fchunk(j, c, lo, n):
            xb = xn2[...]
            g = jnp.dot(xb, wg[c, :, lo:lo + n], preferred_element_type=jnp.float32)
            u = jnp.dot(xb, wu[c, :, lo:lo + n], preferred_element_type=jnp.float32)
            h = (g * u).astype(jnp.bfloat16)
            return lax.dot_general(wd[c, :, lo:lo + n], h, NT_DIMS, preferred_element_type=jnp.float32)

        cp_x(0).wait()
        acc[0] = xin[0].astype(jnp.float32)
        ln1(0)
        cp_qkv().wait()
        for b in range(5):
            nb = min(128, D - b * 128)
            wt[b, :, 0:nb] = wqkv_raw[b * 128:b * 128 + nb, :].astype(jnp.float32).T
        for g, src in enumerate(GROUPS):
            for b in range(5):
                nb = min(128, D - b * 128)
                if src is None:
                    blk = jnp.zeros((H, nb), jnp.bfloat16)
                else:
                    blk = wt[b, pl.ds(src[0] * D + src[1], H, stride=DH), 0:nb].astype(jnp.bfloat16)
                wqkv_p[g * H:(g + 1) * H, b * 128:b * 128 + nb] = blk
        qkv_mm(0)
        cp_wo().wait()
        for t in range(1, NT):
            cp_x(t).wait()
            acc[t] = xin[t].astype(jnp.float32)
        for b in range(5):
            nb = min(128, D - b * 128)
            wt[b, 0:D, 0:nb] = wo_raw[:, b * 128:b * 128 + nb].astype(jnp.float32)
        for b in range(5):
            nb = min(128, D - b * 128)
            rows = [wt[b, pl.ds(d, H, stride=DH), :] for d in range(DH)] + [jnp.zeros((2 * H, 128), jnp.float32)]
            if nb < 128:
                lane = lax.broadcasted_iota(jnp.int32, (H, 128), 1)
                rows = [jnp.where(lane < nb, r_, 0.0) for r_ in rows[:DH]] + rows[DH:]
            wo_p[b * 128:b * 128 + nb, :] = jnp.concatenate(rows, axis=0).T[0:nb, :].astype(jnp.bfloat16)
        def a0(c, carry):
            attn(0, pl.multiple_of(c * 128, 128), 128)
            return carry
        lax.fori_loop(0, TM // 128, a0, 0)
        wo_mm(0); ln1(1)
        qkv_mm(1); ln2(0)

        def job(j, carry):
            ja = jnp.minimum(j + 1, NJ - 1)
            def fbody(c, carry):
                @pl.when(j == 0)
                def _():
                    cp_g(c).wait(); cp_u(c).wait(); cp_d(c).wait()
                r0 = pl.multiple_of(jnp.minimum(c * TA, TM - TA), 16)
                n = FC // NS
                ta = TA // NS
                tot = None
                for s in range(NS):
                    if order == "AF":
                        attn(ja, r0 + s * ta, ta)
                    d = fchunk(j, c, s * n, n)
                    tot = d if tot is None else tot + d
                    if order == "FA":
                        attn(ja, r0 + s * ta, ta)
                acc[tile_of(j)] += tot
                return carry
            lax.fori_loop(0, NF, fbody, 0)

            @pl.when(layer_of(j) == 1)
            def _():
                t = tile_of(j)
                xout[t] = acc[t].astype(jnp.bfloat16)
                cp_o(t).start()

            @pl.when(j < NJ - 1)
            def _():
                wo_mm(j + 1)
                ln1(jnp.minimum(j + 2, NJ - 1))

            @pl.when(j < NJ - 2)
            def _():
                qkv_mm(j + 2)
                ln2(j + 1)

            @pl.when(j == NJ - 2)
            def _():
                ln2(j + 1)
            return carry
        lax.fori_loop(0, NJ, job, 0)
        for t in range(NT):
            cp_o(t).wait()

    def fn(A_x, A_wqkv, A_wo, B_x, B_w_gate, B_w_up, B_w_down):
        xt = A_x.reshape(S, D).T
        hbm = pl.BlockSpec(memory_space=pltpu.MemorySpace.HBM)
        out = pl.pallas_call(
            kernel,
            in_specs=[hbm] * 6,
            out_specs=hbm,
            out_shape=jax.ShapeDtypeStruct((D, S), jnp.bfloat16),
            scratch_shapes=[
                pltpu.VMEM((NT, D, TM), jnp.bfloat16),
                pltpu.VMEM((NT, D, TM), jnp.bfloat16),
                pltpu.VMEM((D, 3 * D), jnp.bfloat16),
                pltpu.VMEM((D, D), jnp.bfloat16),
                pltpu.VMEM((14 * 128, D), jnp.bfloat16),
                pltpu.VMEM((D, DP), jnp.bfloat16),
                pltpu.VMEM((NF, D, FC), jnp.bfloat16),
                pltpu.VMEM((NF, D, FC), jnp.bfloat16),
                pltpu.VMEM((NF, D, FC), jnp.bfloat16),
                pltpu.VMEM((TM, DP), jnp.float32),
                pltpu.VMEM((2, 10, HALO + TM, 128), jnp.float32),
                pltpu.VMEM((NT, D, TM), jnp.float32),
                pltpu.VMEM((TM, D), jnp.bfloat16),
                pltpu.VMEM((TM, D), jnp.bfloat16),
                pltpu.VMEM((TM, DP), jnp.bfloat16),
                pltpu.VMEM((5, 3 * D, 128), jnp.float32),
                pltpu.SemaphoreType.DMA((2 + 3 * NF + 2 * NT,)),
            ],
            compiler_params=pltpu.CompilerParams(
                vmem_limit_bytes=100 * 1024 * 1024, flags=flags),
        )(xt, A_wqkv, A_wo, B_w_gate, B_w_up, B_w_down.T)
        return out.T.reshape(1, S, D)
    return fn


_impl = make(512, 2304, "FA", 1, {"XLA_TPU_EVENLY_DISTRIBUTE_CRITICAL_NODES": True})


@jax.jit
def pallas_interleave_layers__sliding_local_dilated__glu_gated_bilinear__prompt_kernel(
    A_x: jax.Array,
    A_wqkv: jax.Array,
    A_wo: jax.Array,
    B_x: jax.Array,
    B_w_gate: jax.Array,
    B_w_up: jax.Array,
    B_w_down: jax.Array,
):
    return _impl(A_x, A_wqkv, A_wo, B_x, B_w_gate, B_w_up, B_w_down)
```
